```python
import os as _os
_os.environ.setdefault("JAX_PLATFORMS", "cpu")
import jax
import jax.numpy as jnp

def _softmax(x, axis=-1):
    return jax.nn.softmax(x, axis=axis)
def _gelu(x):
    return jax.nn.gelu(x, approximate=True)
def _silu(x):
    return jax.nn.silu(x)
def _sigmoid(x):
    return jax.nn.sigmoid(x)
def _layernorm(x, axis=-1, eps=1e-5):
    m = jnp.mean(x, axis=axis, keepdims=True)
    v = jnp.var(x, axis=axis, keepdims=True)
    return (x - m) / jnp.sqrt(v + eps)
def _scatter_add(tgt, idx, src, axis=0):
    return tgt.at[idx].add(src)
def _segment_sum(src, seg, n):
    return jax.ops.segment_sum(src, seg, n)
class _Rng:
    def __init__(self, key):
        self._k = key
    def _next(self):
        self._k, sub = jax.random.split(self._k)
        return sub
    def normal(self, shape):
        return jax.random.normal(self._next(), shape, dtype=jnp.bfloat16)
    def randint(self, lo, hi, shape):
        return jax.random.randint(self._next(), shape, lo, hi, dtype=jnp.int32)
    def uniform(self, shape, lo=0.0, hi=1.0):
        return jax.random.uniform(self._next(), shape, jnp.bfloat16, lo, hi)
    def permutation(self, n):
        return jax.random.permutation(self._next(), n)


kernel_name = 'concat_heads__mha_block__linear_attn_block__prompt'

def setup_inputs():
    _rng = _Rng(jax.random.key(int.from_bytes(__import__("os").urandom(4), "little")))
    _w = (lambda a: (lambda t: t.astype(jnp.bfloat16) if jnp.issubdtype(t.dtype, jnp.floating) else t)(jnp.asarray(a)))
    def _A_setup():
        B, S, D, H = 1, 2048, 1024, 32
        return {
            "x": _w((lambda *s: _rng.normal(s) * 0.2)(B, S, D)),
            "wqkv": _w((lambda *s: _rng.normal(s) * 0.2)(D, 3 * D)),
            "wo": _w((lambda *s: _rng.normal(s) * 0.05)(D, D)),
        }
    _A_in = _A_setup()

    def _B_setup():
        B, S, D = 1, 2048, 1024
        return {
            "x": _w((lambda *s: _rng.normal(s) * 0.05)(B, S, D)),
            "wqkv": _w((lambda *s: _rng.normal(s) * 1.6)(D, 3 * D)),
            "wo": _w((lambda *s: _rng.normal(s) * 0.1)(D, D)),
        }
    _B_in = _B_setup()

    return {
        "A_x": _A_in["x"],
        "A_wqkv": _A_in["wqkv"],
        "A_wo": _A_in["wo"],
        "B_x": _B_in["x"],
        "B_wqkv": _B_in["wqkv"],
        "B_wo": _B_in["wo"],
    }

def reference(A_x, A_wqkv, A_wo, B_x, B_wqkv, B_wo):
    def _A_ref(x, wqkv, wo):
        B, S, D = x.shape
        H = 32
        Dh = D // H
        qkv = (lambda x, *d: x.transpose(*d))((x @ wqkv).reshape(B, S, 3, H, Dh), 2, 0, 3, 1, 4)
        q, k, v = qkv[0], qkv[1], qkv[2]
        scores = jnp.einsum("bhqd,bhkd->bhqk", q, k) * (Dh ** -0.5)
        p = _softmax(scores, axis=-1)
        o = jnp.einsum("bhqk,bhkd->bhqd", p, v)
        return (lambda x, *d: x.transpose(*d))(o, 0, 2, 1, 3).reshape(B, S, D) @ wo

    def _B_ref(x, wqkv, wo):
        B, S, D = x.shape
        H = 32; Dh = D // H
        qkv = (lambda x, *d: x.transpose(*d))((x @ wqkv).reshape(B, S, 3, H, Dh), 2, 0, 3, 1, 4)
        q, k, v = qkv[0], qkv[1], qkv[2]
        phi = lambda t: jnp.where(t > 0, t + 1, jnp.exp(t)) + 1e-6
        pq, pk = phi(q), phi(k)
        kv = jnp.einsum("bhsd,bhse->bhde", pk, v)
        z = jnp.einsum("bhsd->bhd", pk)
        num = jnp.einsum("bhqd,bhde->bhqe", pq, kv)
        den = jnp.einsum("bhqd,bhd->bhq", pq, z)[..., None] + 1e-6
        o = num / den
        return (lambda x, *d: x.transpose(*d))(o, 0, 2, 1, 3).reshape(B, S, D) @ wo

    a = _A_ref(A_x, A_wqkv, A_wo)
    b = _B_ref(B_x, B_wqkv, B_wo)
    return jnp.concatenate([a, b], axis=-1)
```

```python
import math

import jax
import jax.numpy as jnp
from jax import lax
from jax.experimental import pallas as pl
from jax.experimental.pallas import tpu as pltpu

S, D, H, DH = 2048, 1024, 32, 32
HF = 512
NSC = S // (2 * HF)
QB = HF
NQ = S // QB
NB = H * NQ
CH = 128
NC = S // CH
LAG = 2
GATE_ROWS, GATE_LEAD = 32, 168
LOOPS = ((10, 11), (8, 2))
QSCALE = (DH ** -0.5) * math.log2(math.e)
f32, bf16, u32 = jnp.float32, jnp.bfloat16, jnp.uint32

SUMS = (((0, 0), 1, (1, 1)), ((1, 0), 1, (1, 1)), ((0, 0), 1, (0, 1)),
        ((1, 0), -1, (0, 0)), ((0, 1), -1, (1, 1)))
LSUM_OF = {1: 0, 2: 1, 5: 2, 6: 3, 7: 4}
RSUM_OF = {1: 0, 7: 1, 6: 2, 4: 3, 3: 4}
LQUAD_OF = {3: (0, 0), 4: (1, 1)}
RQUAD_OF = {2: (0, 0), 5: (1, 1)}
COMBINE = {(1, 0): (2, 4), (1, 1): (1, -2, 3, 6), (0, 0): (1, 4, -5, 7), (0, 1): (3, 5)}


def _pack(x):
    return pltpu.bitcast(x.astype(bf16), u32)


def _unpack(x):
    return pltpu.bitcast(x, bf16)


def _dot(a, b):
    return jnp.dot(a, b, preferred_element_type=f32)


def _dot_t(at, b):
    return lax.dot_general(at, b, (((0,), (0,)), ((), ())), preferred_element_type=f32)


def _phi(t):
    return jnp.where(t > 0, t + 1.0, jnp.exp(t)) + 1e-6


def _recip(x):
    r = pl.reciprocal(x, approx=True)
    return r * (2.0 - x * r)


def _cut(i, n=HF):
    return slice(i * n, (i + 1) * n)


def _head_rows(h):
    return pl.ds(pl.multiple_of(h * (DH // 2), DH // 2), DH // 2)


def _strassen(lq, lsums, rq, rsums, emit, *, make_l, make_r, dot=_dot, extra=None,
              order=(2, 4, 3, 5, 6, 1, 7)):
    def quad_sum(quad, dst, n):
        a, sign, b = SUMS[n]
        x, y = quad(*a).astype(f32), quad(*b).astype(f32)
        dst[n][...] = _pack(x + y if sign > 0 else x - y)

    prod, out = {}, {}
    for p in order:
        if extra:
            extra(p)
        if make_l and p in LSUM_OF:
            quad_sum(lq, lsums, LSUM_OF[p])
        if make_r and p in RSUM_OF:
            quad_sum(rq, rsums, RSUM_OF[p])
        prod[p] = dot(_unpack(lsums[LSUM_OF[p]][...]) if p in LSUM_OF else lq(*LQUAD_OF[p]),
                      _unpack(rsums[RSUM_OF[p]][...]) if p in RSUM_OF else rq(*RQUAD_OF[p]))
        for ij, terms in COMBINE.items():
            if p in terms:
                out[ij] = out[ij] + prod[p] if ij in out else prod[p]
            elif -p in terms:
                out[ij] = out[ij] - prod[p] if ij in out else -prod[p]
            else:
                continue
            if all(abs(q) in prod for q in terms):
                emit(*ij, out[ij])


def _kernel(xa_h, wa_h, woa_h, xb_h, wb_h, wob_h, out_h,
            xa, wa, woa, xb, wb, wob, k4, qt, vt, ot, s_even, s_odd, sems, osems,
            xs, ws, os_, pkt, pqt, kv, mo, zc):
    def copy(src, dst, idx, sem):
        return pltpu.make_async_copy(src.at[idx], dst.at[idx], sems.at[sem])

    cp_x = [copy(xa_h, xa, (_cut(0), _cut(0)), 0), copy(xa_h, xa, (_cut(1),), 1),
            copy(xa_h, xa, (_cut(0), _cut(1)), 2), copy(xa_h, xa, (_cut(1, 2 * HF),), 3)]
    cp_wq = {(i, j): copy(wa_h, wa, (_cut(i), _cut(j)), 4 + 2 * i + j)
             for i in range(2) for j in range(2)}
    cp_wk = copy(wa_h, wa, (slice(None), _cut(1, D)), 8)
    cp_wv = copy(wa_h, wa, (slice(None), _cut(2, D)), 9)
    late = [pltpu.make_async_copy(src, dst, sems.at[10 + n])
            for n, (src, dst) in enumerate(((woa_h, woa), (xb_h, xb), (wb_h, wb), (wob_h, wob)))]
    feed = {(0, 0, 2): ([cp_x[1], cp_wq[0, 0], cp_wq[1, 0]], [cp_x[0], cp_wq[0, 1], cp_wq[1, 1]]),
            (0, 0, 3): ([cp_x[0], cp_wq[0, 1], cp_wq[1, 1]], [cp_x[2], cp_wk]),
            (0, 0, 1): ([cp_x[2]], []),
            (0, 0, 5): ([cp_wk], [cp_wv, cp_x[3]]),
            (0, 1, 6): ([cp_wv, cp_x[3]], [])}
    for c in feed[0, 0, 2][0]:
        c.start()

    def xquad(x, sc):
        return lambda i, j: x[_cut(2 * sc + i), _cut(j)]

    def wquad(w, part):
        return lambda i, j: w[_cut(i), _cut(2 * part + j)]

    for sc in range(NSC):
        def emit_q(i, j, y):
            qt[2 * sc + i, _cut(j, HF // 2), :] = _pack((y * QSCALE).T)

        def emit_k(i, j, y):
            kp = _pack(y)
            for g in range(HF // 128):
                kg = kp[:, _cut(g, 128)]
                for e in range(128 // DH):
                    k4[(j * HF + g * 128) // DH + e, _cut(2 * sc + i, HF // 2), :] = (
                        kg if e == 0 else pltpu.roll(kg, 128 - DH * e, 1))

        def emit_v(i, j, y):
            vt[2 * sc + i, _cut(j, HF // 2), :] = _pack(y.T)

        for part, emit in enumerate((emit_q, emit_k, emit_v)):
            def release(p):
                done, nxt = feed.get((sc, part, p), ((), ()))
                for c in done:
                    c.wait()
                for c in nxt:
                    c.start()
            first = dict(order=(2, 4, 3, 6, 1, 7, 5)) if (sc, part) == (0, 0) else {}
            _strassen(xquad(xa, sc), xs[sc], wquad(wa, part), ws[part], emit,
                      make_l=part == 0, make_r=sc == 0, extra=release, **first)

    sbuf = (s_even, s_odd)

    def qk_slot(b, par, c, m_new):
        h, qb = b // NQ, b % NQ
        s = _dot(_unpack(k4[h, _cut(c, CH // 2), :])[:, :DH], _unpack(qt[qb, _head_rows(h), :]))
        sbuf[par][_cut(c, CH), :] = s
        run = []
        for r in range(0, CH, 8):
            m_new = s[r:r + 8] if (c == 0 and r == 0) else jnp.maximum(m_new, s[r:r + 8])
            run.append(m_new)
        return run

    def pv_slot(b, par, c, m_cur, l, acc, gate):
        h, qb = b // NQ, b % NQ
        ps = []
        for r in range(0, CH, GATE_ROWS):
            g = gate(r)
            mg = m_cur if g is None else jnp.maximum(m_cur, jnp.minimum(m_cur, g))
            for t in range(r, r + GATE_ROWS, 8):
                p = jnp.exp2(sbuf[par][c * CH + t:c * CH + t + 8, :] - mg)
                l = p if (c == 0 and t == 0) else l + p
                ps.append(p)
        cr, cc = divmod(c * CH, HF)
        pv = _dot(_unpack(vt[cr, _head_rows(h), cc:cc + CH]), jnp.concatenate(ps, axis=0).astype(bf16))
        acc = pv if c == 0 else acc + pv
        if c == NC - 1:
            ot[qb, _head_rows(h), :] = _pack(acc / jnp.sum(l, axis=0, keepdims=True))
        return l, acc

    def slots(b0, t0, t1, state, do_qk=True, do_pv=True):
        m_new, m_rdy, m_cur, l, acc = state
        run = {}
        for t in range(t0, t1):
            if do_qk:
                j, c = divmod(t, NC)
                rr = qk_slot(b0 + j, j % 2, c, m_new)
                m_new = rr[-1]
                for i, v in enumerate(rr):
                    run[t * CH + 8 * i] = v
                if c == NC - 1:
                    m_rdy = jnp.broadcast_to(jnp.max(m_new, axis=0, keepdims=True), (8, QB))
            if do_pv:
                j, c = divmod(t - NC - LAG, NC)
                if c == 0:
                    m_cur = m_rdy
                l, acc = pv_slot(b0 + j, j % 2, c, m_cur, l, acc,
                                 lambda r: run.get(t * CH + r - GATE_LEAD))
        return m_new, m_rdy, m_cur, l, acc

    zero = jnp.zeros((8, QB), f32)
    state = slots(0, 0, NC + LAG, (zero, zero, zero, zero, jnp.zeros((DH, QB), f32)), do_pv=False)
    state = slots(0, NC + LAG, 2 * NC, state)
    b0 = 2
    for u, n in LOOPS:
        def body(j, st, b0=b0, u=u):
            if b0 == 2:
                @pl.when(j == 0)
                def _():
                    for c in late:
                        c.start()
            return slots(b0 + j * u, 0, u * NC, st)
        state = lax.fori_loop(0, n, body, state)
        b0 += u * n
    assert b0 == NB
    for c in late:
        c.wait()
    slots(NB, 0, NC + LAG, state, do_qk=False)

    out_cps = []

    def out_proj(lq, w, sc, half):
        def emit(i, j, y):
            r, c = (2 * sc + i, j) if half == 0 else (i, 2 * sc + j)
            n = 4 if (half, sc, i, j) == (1, NSC - 1, 0, 0) else 1
            for e in range(n):
                buf = (wa if half else xa).at[_cut(r), _cut(n * c + e, HF // n)]
                buf[...] = y[:, _cut(e, HF // n)].astype(bf16)
                cp = pltpu.make_async_copy(
                    buf, out_h.at[_cut(2 * sc + i), _cut(n * (2 * half + j) + e, HF // n)],
                    osems.at[len(out_cps)])
                cp.start()
                out_cps.append(cp)
        _strassen(lq, os_[sc], wquad(w, 0), ws[6 + half], emit,
                  make_l=True, make_r=sc == 0, dot=_dot_t)

    for sc in range(NSC):
        out_proj(lambda i, j: _unpack(ot[2 * sc + i, _cut(j, HF // 2), :]), woa, sc, 0)

    def project_b(sc, part, emit, extra=None):
        _strassen(xquad(xb, sc), xs[2 + sc], wquad(wb, part), ws[3 + part], emit,
                  make_l=part == 1, make_r=sc == 0, extra=extra)

    z = [jnp.zeros((8, HF), f32), jnp.zeros((8, HF), f32)]
    for sc in range(NSC):
        def emit_pk(i, j, y):
            pk = _phi(y)
            z[j] = z[j] + jnp.sum(pk.reshape(HF // 8, 8, HF), axis=0)
            pkt[2 * sc + i][j][...] = _pack(pk.T)
        project_b(sc, 1, emit_pk)
    for n in range(D // 128):
        j, g = divmod(n, HF // 128)
        zrow = jnp.sum(z[j][:, _cut(g, 128)], axis=0, keepdims=True)
        zc[n] = jnp.broadcast_to(zrow, (128, 128)).T

    for sc in range(NSC):
        def emit_kv(i, j, y):
            v = y.astype(bf16)
            for g in range(HF // 128):
                n = j * (HF // 128) + g
                t = _dot(_unpack(pkt[2 * sc + i][j][_cut(g, 64), :]), v[:, _cut(g, 128)])
                kv[n][...] = t if (sc == 0 and i != j) else kv[n][...] + t
        project_b(sc, 2, emit_kv)

    def fold_state(p):
        if p == 3:
            same = ((lax.broadcasted_iota(jnp.int32, (128, 128), 0) >> 5)
                    == (lax.broadcasted_iota(jnp.int32, (128, 128), 1) >> 5))
            for n in range(D // 128):
                mean_v = jnp.where(same, kv[n][...] * _recip(zc[n]), 0.0).astype(bf16)
                mo[_cut(n, 128), :] = _dot(mean_v, wob[_cut(n, 128), :]).astype(bf16)

    for sc in range(NSC):
        def emit_pq(i, j, y):
            pt = _phi(y).T
            rows = []
            for e in range(HF // DH):
                g, r = divmod(j * HF + e * DH, 128)
                t = pt[_cut(e, DH)] * jnp.concatenate([zc[g, r:r + DH, :]] * (HF // 128), axis=1)
                rows.append(t * _recip(jnp.sum(t, axis=0, keepdims=True) + 1e-6))
            pqt[2 * sc + i][j][...] = _pack(jnp.concatenate(rows, axis=0))
        project_b(sc, 0, emit_pq, fold_state if sc == 0 else None)

    for sc in range(NSC):
        out_proj(lambda i, j: _unpack(pqt[2 * sc + i][j][...]), mo, sc, 1)
    for c in out_cps:
        c.wait()


@jax.jit
def pallas_concat_heads__mha_block__linear_attn_block__prompt_kernel(A_x, A_wqkv, A_wo, B_x, B_wqkv, B_wo):
    quad = pltpu.VMEM((HF // 2, HF), u32)
    rows_t = pltpu.VMEM((NQ, D // 2, QB), u32)
    inputs = [pltpu.VMEM((S, D), bf16), pltpu.VMEM((D, 3 * D), bf16), pltpu.VMEM((D, D), bf16)]
    out = pl.pallas_call(
        _kernel,
        out_shape=jax.ShapeDtypeStruct((S, 2 * D), bf16),
        in_specs=[pl.BlockSpec(memory_space=pl.ANY)] * 6,
        out_specs=pl.BlockSpec(memory_space=pl.ANY),
        scratch_shapes=inputs + inputs + [
            pltpu.VMEM((H, S // 2, 128), u32),
            rows_t, rows_t, rows_t,
            pltpu.VMEM((S, QB), f32), pltpu.VMEM((S, QB), f32),
            pltpu.SemaphoreType.DMA((14,)), pltpu.SemaphoreType.DMA((19,)),
            [[quad] * 5] * 4, [[quad] * 5] * 8, [[quad] * 5] * 2,
            [[quad] * 2] * 4, [[quad] * 2] * 4,
            [pltpu.VMEM((128, 128), f32)] * (D // 128),
            pltpu.VMEM((D, D), bf16),
            pltpu.VMEM((D // 128, 128, 128), f32),
        ],
        compiler_params=pltpu.CompilerParams(vmem_limit_bytes=120 * 2**20),
        name="fused_mha_linattn",
    )(A_x.reshape(S, D), A_wqkv, A_wo, B_x.reshape(S, D), B_wqkv, B_wo)
    return out.reshape(1, S, 2 * D)
```
